```python
import os as _os
_os.environ.setdefault("JAX_PLATFORMS", "cpu")
import jax
import jax.numpy as jnp

def _softmax(x, axis=-1):
    return jax.nn.softmax(x, axis=axis)
def _gelu(x):
    return jax.nn.gelu(x, approximate=True)
def _silu(x):
    return jax.nn.silu(x)
def _sigmoid(x):
    return jax.nn.sigmoid(x)
def _layernorm(x, axis=-1, eps=1e-5):
    m = jnp.mean(x, axis=axis, keepdims=True)
    v = jnp.var(x, axis=axis, keepdims=True)
    return (x - m) / jnp.sqrt(v + eps)
def _scatter_add(tgt, idx, src, axis=0):
    return tgt.at[idx].add(src)
def _segment_sum(src, seg, n):
    return jax.ops.segment_sum(src, seg, n)
class _Rng:
    def __init__(self, key):
        self._k = key
    def _next(self):
        self._k, sub = jax.random.split(self._k)
        return sub
    def normal(self, shape):
        return jax.random.normal(self._next(), shape, dtype=jnp.bfloat16)
    def randint(self, lo, hi, shape):
        return jax.random.randint(self._next(), shape, lo, hi, dtype=jnp.int32)
    def uniform(self, shape, lo=0.0, hi=1.0):
        return jax.random.uniform(self._next(), shape, jnp.bfloat16, lo, hi)
    def permutation(self, n):
        return jax.random.permutation(self._next(), n)


kernel_name = 'concat_heads__gqa_block_cached__sliding_block_cached__decode'

def setup_inputs():
    _rng = _Rng(jax.random.key(int.from_bytes(__import__("os").urandom(4), "little")))
    _w = (lambda a: (lambda t: t.astype(jnp.bfloat16) if jnp.issubdtype(t.dtype, jnp.floating) else t)(jnp.asarray(a)))
    def _A_setup():
        B, Sq, D = 2, 1, 448
        Hq, Hkv, Sk, Dh = 16, 8, 8192, 256
        assert Hq % Hkv == 0, (Hq, Hkv)
        return {
            "x": _w((lambda *s: _rng.normal(s) * 0.8)(B, Sq, D)),
            "k_cache": _w((lambda *s: _rng.normal(s) * 0.8)(B, Hkv, Sk, Dh)),
            "v_cache": _w((lambda *s: _rng.normal(s) * 0.05)(B, Hkv, Sk, Dh)),
            "wq": _w((lambda *s: _rng.normal(s) * 0.8)(D, Hq * Dh) * (D ** -0.5)),
            "wo": _w((lambda *s: _rng.normal(s) * 0.05)(Hq * Dh, D) * ((Hq * Dh) ** -0.5)),
        }
    _A_in = _A_setup()

    def _B_setup():
        B, Sq, D = 2, 1, 448
        Hq, Hkv, Sk, Dh = 16, 8, 8192, 256
        assert Hq % Hkv == 0, (Hq, Hkv)
        return {
            "x": _w((lambda *s: _rng.normal(s) * 0.8)(B, Sq, D)),
            "k_cache": _w((lambda *s: _rng.normal(s) * 0.8)(B, Hkv, Sk, Dh)),
            "v_cache": _w((lambda *s: _rng.normal(s) * 0.05)(B, Hkv, Sk, Dh)),
            "wq": _w((lambda *s: _rng.normal(s) * 0.8)(D, Hq * Dh) * (D ** -0.5)),
            "wo": _w((lambda *s: _rng.normal(s) * 0.05)(Hq * Dh, D) * ((Hq * Dh) ** -0.5)),
        }
    _B_in = _B_setup()

    return {
        "A_x": _A_in["x"],
        "A_k_cache": _A_in["k_cache"],
        "A_v_cache": _A_in["v_cache"],
        "A_wq": _A_in["wq"],
        "A_wo": _A_in["wo"],
        "B_x": _B_in["x"],
        "B_k_cache": _B_in["k_cache"],
        "B_v_cache": _B_in["v_cache"],
        "B_wq": _B_in["wq"],
        "B_wo": _B_in["wo"],
    }

def reference(A_x, A_k_cache, A_v_cache, A_wq, A_wo, B_x, B_k_cache, B_v_cache, B_wq, B_wo):
    def _A_ref(x, k_cache, v_cache, wq, wo):
        B, Sq, D = x.shape
        Hq, Dh = 16, 256
        Hkv = k_cache.shape[1]
        rep = Hq // Hkv
        q = (lambda x, *d: x.transpose(*d))((x @ wq).reshape(B, Sq, Hq, Dh), 0, 2, 1, 3)
        k = jnp.repeat(k_cache, rep, axis=1)
        v = jnp.repeat(v_cache, rep, axis=1)
        scores = jnp.einsum("bhqd,bhkd->bhqk", q, k) * (Dh ** -0.5)
        p = _softmax(scores, axis=-1)
        o = jnp.einsum("bhqk,bhkd->bhqd", p, v)
        return (lambda x, *d: x.transpose(*d))(o, 0, 2, 1, 3).reshape(B, Sq, Hq * Dh) @ wo

    def _B_ref(x, k_cache, v_cache, wq, wo):
        B, Sq, D = x.shape
        Hq, Dh = 16, 256
        Hkv, Sk = k_cache.shape[1], k_cache.shape[2]
        W = min(4096, max(256, Sk // 4))
        rep = Hq // Hkv
        q = (lambda x, *d: x.transpose(*d))((x @ wq).reshape(B, Sq, Hq, Dh), 0, 2, 1, 3)
        k = jnp.repeat(k_cache[:, :, Sk - W:, :], rep, axis=1)
        v = jnp.repeat(v_cache[:, :, Sk - W:, :], rep, axis=1)
        scores = jnp.einsum("bhqd,bhkd->bhqk", q, k) * (Dh ** -0.5)
        p = _softmax(scores, axis=-1)
        o = jnp.einsum("bhqk,bhkd->bhqd", p, v)
        return (lambda x, *d: x.transpose(*d))(o, 0, 2, 1, 3).reshape(B, Sq, Hq * Dh) @ wo

    a = _A_ref(A_x, A_k_cache, A_v_cache, A_wq, A_wo)
    b = _B_ref(B_x, B_k_cache, B_v_cache, B_wq, B_wo)
    return jnp.concatenate([a, b], axis=-1)
```

```python
import jax
import jax.numpy as jnp
from jax import lax
import jax.experimental.pallas as pl
import jax.experimental.pallas.tpu as pltpu

_NT = (((1,), (1,)), ((), ()))
_NN = (((1,), (0,)), ((), ()))
_ROWS = 8


def build(NS=4, BLK=128, SUB=64, R=4, mode="kvs", name="attn_decode", nobc=True, wsplit=2):
    def fn(A_x, A_k_cache, A_v_cache, A_wq, A_wo, B_x, B_k_cache, B_v_cache, B_wq, B_wo):
        B, Sq, D = A_x.shape
        Hq, Dh = 16, 256
        Hkv, SkA = A_k_cache.shape[1], A_k_cache.shape[2]
        SkB = B_k_cache.shape[2]
        W = min(4096, max(256, SkB // 4))
        rep = Hq // Hkv
        assert B == 2 and Sq == 1 and rep == 2
        HD = Hq * Dh
        GW = rep * Dh
        scale = Dh ** -0.5
        CH = NS * BLK
        ncA, ncB = SkA // CH, W // CH
        NB_, NA_ = Hkv * ncB, Hkv * ncA
        NTOT = NA_ + NB_
        WB = 8
        nwb = D // WB

        def kernel(xa_hbm, ka_hbm, va_hbm, wqa_hbm, woa_hbm,
                   xb_hbm, kb_hbm, vb_hbm, wqb_hbm, wob_hbm, out_ref,
                   k_buf, v_buf, x_buf, wq_buf, wo_buf, q_scr, o_scr,
                   kv_sem, x_sem, w_sem, woa_sem):
            branches = (
                (ka_hbm, va_hbm, ncA, 0, SkA),
                (kb_hbm, vb_hbm, ncB, SkB - W, W),
            )

            def start_chunk(br, u, slot):
                k_hbm, v_hbm, nc, row0, nrows = branches[br]
                g, j = lax.div(u, nc), lax.rem(u, nc)
                stride = nrows // NS
                span = (NS - 1) * stride + BLK
                base = pl.multiple_of(row0 + j * BLK, BLK)
                src = [[h.at[b, g, pl.ds(base, span)] for b in range(B)] for h in (k_hbm, v_hbm)]
                dst = [[h.at[slot, b] for b in range(B)] for h in (k_buf, v_buf)]

                def cp(w, b, s, o, prio):
                    pltpu.make_async_copy(
                        src[w][b].at[pl.ds(s * stride + o, SUB)],
                        dst[w][b].at[pl.ds(s * BLK + o, SUB)],
                        kv_sem.at[slot, w]).start(priority=prio)

                if mode == "kv":
                    for s in range(NS):
                        for b in range(B):
                            for o in range(0, BLK, SUB):
                                cp(0, b, s, o, 0)
                                cp(1, b, s, o, 1)
                elif mode == "kvs":
                    for s in range(NS):
                        for b in range(B):
                            for o in range(0, BLK, SUB):
                                cp(0, b, s, o, 0)
                                cp(1, b, (s + NS // 2) % NS, o, 1)
                elif mode == "bb":
                    for w in range(2):
                        for s in range(NS):
                            for o in range(0, BLK, SUB):
                                cp(w, 0, s, o, 0)
                                cp(w, 1, s, o, 1)
                elif mode == "ss":
                    for w in range(2):
                        for b in range(B):
                            for s in range(0, NS, 2):
                                for o in range(0, BLK, SUB):
                                    cp(w, b, s, o, 0)
                                    cp(w, b, s + 1, o, 1)
                elif mode == "p0":
                    for w in range(2):
                        for b in range(B):
                            for s in range(NS):
                                for o in range(0, BLK, SUB):
                                    cp(w, b, s, o, 0)

            def start_wpair(src0, dst0, sem0, blk0, src1, dst1, sem1, blk1):
                r0 = pl.multiple_of(blk0 * WB, WB)
                r1 = pl.multiple_of(blk1 * WB, WB)
                cw = HD // wsplit
                for c in range(wsplit):
                    pltpu.make_async_copy(src0.at[pl.ds(r0, WB), pl.ds(c * cw, cw)],
                                          dst0.at[pl.ds(r0, WB), pl.ds(c * cw, cw)], sem0).start(priority=0)
                    pltpu.make_async_copy(src1.at[pl.ds(r1, WB), pl.ds(c * cw, cw)],
                                          dst1.at[pl.ds(r1, WB), pl.ds(c * cw, cw)], sem1).start(priority=1)

            def start_rows(src, dst, sem, first, count, nstream):
                per = count // nstream

                def body(i, _):
                    for s in range(0, nstream, 2):
                        start_wpair(src, dst, sem, first + s * per + i,
                                    src, dst, sem, first + (s + 1) * per + i)
                lax.fori_loop(0, per, body, None)

            tiles = [(lo, min(lo + 128, D)) for lo in range(0, D, 128)]

            def start_woa(n):
                lo, hi = tiles[n]
                start_rows(woa_hbm, wo_buf.at[0], woa_sem.at[n], lo // WB, (hi - lo) // WB, 4)

            def start_step(t):
                slot = lax.rem(t, R)

                @pl.when(t < NB_)
                def _():
                    start_chunk(1, t, slot)

                @pl.when(jnp.logical_and(t >= NB_, t < NTOT))
                def _():
                    start_chunk(0, t - NB_, slot)

                for n in range(min(R - 1, len(tiles))):
                    pl.when(t == NTOT + n)(lambda n=n: start_woa(n))

            x_copies = [
                pltpu.make_async_copy(xa_hbm, x_buf.at[0], x_sem.at[0]),
                pltpu.make_async_copy(xb_hbm, x_buf.at[1], x_sem.at[1]),
            ]
            start_rows(wqb_hbm, wq_buf.at[1], w_sem.at[1], 0, nwb, 8)
            for c in x_copies:
                c.start()
            start_rows(wqa_hbm, wq_buf.at[0], w_sem.at[0], 0, nwb, 8)
            start_rows(wob_hbm, wo_buf.at[1], w_sem.at[2], 0, nwb, 8)

            def warm(t, _):
                start_chunk(1, t, t)
            lax.fori_loop(0, R - 1, warm, None)

            def row_ids(n):
                return lax.broadcasted_iota(jnp.int32, (_ROWS, n), 0)

            def project_q(br):
                x_copies[br].wait()
                x = x_buf[br].astype(jnp.float32)
                xr = jnp.where(row_ids(D) % 2 == 0,
                               jnp.broadcast_to(x[0:1], (_ROWS, D)),
                               jnp.broadcast_to(x[1:2], (_ROWS, D))).astype(jnp.bfloat16)
                pltpu.make_async_copy(wq_buf.at[br], wq_buf.at[br], w_sem.at[br]).wait()

                def body(g, _):
                    cols = pl.ds(pl.multiple_of(g * GW, GW), GW)
                    q = lax.dot_general(xr, wq_buf[br, :, cols], _NN,
                                        preferred_element_type=jnp.float32)
                    q_scr[br, g] = jnp.where((row_ids(Dh) // 2) % 2 == 0, q[:, :Dh], q[:, Dh:])
                lax.fori_loop(0, Hkv, body, None)

            def attend(br, first):
                nc = branches[br][2]

                def group_body(g, _):
                    q = q_scr[br, g].astype(jnp.bfloat16)

                    def chunk_body(j, carry):
                        m, l, acc = carry
                        t = first + g * nc + j
                        slot = lax.rem(t, R)
                        start_step(t + (R - 1))
                        pltpu.make_async_copy(k_buf.at[slot], k_buf.at[slot], kv_sem.at[slot, 0]).wait()
                        pltpu.make_async_copy(v_buf.at[slot], v_buf.at[slot], kv_sem.at[slot, 1]).wait()
                        s0, s1 = [lax.dot_general(q, k_buf[slot, b], _NT,
                                                  preferred_element_type=jnp.float32) for b in range(B)]
                        s = jnp.where(row_ids(CH) % 2 == 0, s0, s1) * scale
                        m_new = jnp.maximum(m, jnp.max(s, axis=-1, keepdims=True))
                        alpha = jnp.exp(m - m_new)
                        p = jnp.exp(s - m_new)
                        l = alpha * l + jnp.sum(p, axis=-1, keepdims=True)
                        pb = p.astype(jnp.bfloat16)
                        o0, o1 = [lax.dot_general(pb, v_buf[slot, b], _NN,
                                                  preferred_element_type=jnp.float32) for b in range(B)]
                        acc = alpha * acc + jnp.where(row_ids(Dh) % 2 == 0, o0, o1)
                        return m_new, l, acc

                    init = (jnp.full((_ROWS, 1), -jnp.inf, jnp.float32),
                            jnp.zeros((_ROWS, 1), jnp.float32),
                            jnp.zeros((_ROWS, Dh), jnp.float32))
                    _, l, acc = lax.fori_loop(0, nc, chunk_body, init)
                    o = acc / l
                    c0 = pl.multiple_of(g * GW, GW)
                    o_scr[br, :, pl.ds(c0, Dh)] = o
                    o_scr[br, :, pl.ds(c0 + Dh, Dh)] = pltpu.roll(o, _ROWS - 2, 0)

                lax.fori_loop(0, Hkv, group_body, None)

            project_q(1)
            project_q(0)
            attend(1, 0)
            pltpu.make_async_copy(wo_buf.at[1], wo_buf.at[1], w_sem.at[2]).wait()
            res = lax.dot_general(o_scr[1].astype(jnp.bfloat16), wo_buf[1], _NT,
                                  preferred_element_type=jnp.float32)
            out_ref[:, D:2 * D] = res[0:B].astype(out_ref.dtype)
            attend(0, NB_)
            for n in range(R - 1, len(tiles)):
                start_woa(n)
            oa = o_scr[0].astype(jnp.bfloat16)
            for n, (lo, hi) in enumerate(tiles):
                piece = wo_buf.at[0, pl.ds(lo, hi - lo)]
                pltpu.make_async_copy(piece, piece, woa_sem.at[n]).wait()
                res = lax.dot_general(oa, piece[...], _NT, preferred_element_type=jnp.float32)
                out_ref[:, lo:hi] = res[0:B].astype(out_ref.dtype)

        hbm = pl.BlockSpec(memory_space=pltpu.HBM)
        out = pl.pallas_call(
            kernel,
            out_shape=jax.ShapeDtypeStruct((B, 2 * D), A_x.dtype),
            in_specs=[hbm] * 10,
            out_specs=pl.BlockSpec(memory_space=pltpu.VMEM),
            scratch_shapes=[
                pltpu.VMEM((R, B, CH, Dh), A_k_cache.dtype),
                pltpu.VMEM((R, B, CH, Dh), A_v_cache.dtype),
                pltpu.VMEM((2, B, D), A_x.dtype),
                pltpu.VMEM((2, D, HD), A_wq.dtype),
                pltpu.VMEM((2, D, HD), A_wo.dtype),
                pltpu.VMEM((2, Hkv, _ROWS, Dh), jnp.float32),
                pltpu.VMEM((2, _ROWS, HD), jnp.float32),
                pltpu.SemaphoreType.DMA((R, 2)),
                pltpu.SemaphoreType.DMA((2,)),
                pltpu.SemaphoreType.DMA((3,)),
                pltpu.SemaphoreType.DMA((4,)),
            ],
            compiler_params=pltpu.CompilerParams(vmem_limit_bytes=100 * 2**20, disable_bounds_checks=nobc),
            name=name,
        )(A_x.reshape(B, D), A_k_cache, A_v_cache, A_wq, A_wo.T,
          B_x.reshape(B, D), B_k_cache, B_v_cache, B_wq, B_wo.T)
        return out.reshape(B, Sq, 2 * D)
    return jax.jit(fn)


pallas_concat_heads__gqa_block_cached__sliding_block_cached__decode_kernel = build()
```

```python
import jax
import jax.numpy as jnp
from jax import lax
import jax.experimental.pallas as pl
import jax.experimental.pallas.tpu as pltpu

_NT = (((1,), (1,)), ((), ()))
_NN = (((1,), (0,)), ((), ()))
_ROWS = 8


def build(NS=4, BLK=128, SUB=64, R=7, mode="kv", name="k5", nobc=True, SH=96, WSH=3072, rev=True):
    def fn(A_x, A_k_cache, A_v_cache, A_wq, A_wo, B_x, B_k_cache, B_v_cache, B_wq, B_wo):
        B, Sq, D = A_x.shape
        Hq, Dh = 16, 256
        Hkv, SkA = A_k_cache.shape[1], A_k_cache.shape[2]
        SkB = B_k_cache.shape[2]
        W = min(4096, max(256, SkB // 4))
        rep = Hq // Hkv
        assert B == 2 and Sq == 1 and rep == 2
        HD = Hq * Dh
        GW = rep * Dh
        scale = Dh ** -0.5
        CH = NS * BLK
        ncA, ncB = SkA // CH, W // CH
        NB_, NA_ = Hkv * ncB, Hkv * ncA
        NTOT = NA_ + NB_
        WB = 8
        nwb = D // WB

        def kernel(xa_hbm, ka_hbm, va_hbm, wqa_hbm, woa_hbm,
                   xb_hbm, kb_hbm, vb_hbm, wqb_hbm, wob_hbm, out_ref,
                   k_buf, v_buf, x_buf, wq_buf, wo_buf, q_scr, o_scr,
                   kv_sem, x_sem, w_sem, woa_sem):
            branches = (
                (ka_hbm, va_hbm, ncA, 0, SkA),
                (kb_hbm, vb_hbm, ncB, SkB - W, W),
            )

            def pieces(wrap):
                cuts = set(range(0, BLK, SUB)) | ({BLK - SH} if wrap and SH else set())
                cuts = sorted(cuts) + [BLK]
                return [(lo, hi - lo) for lo, hi in zip(cuts[:-1], cuts[1:])]

            def start_chunk(br, u, slot):
                k_hbm, v_hbm, nc, row0, nrows = branches[br]
                g, j = lax.div(u, nc), lax.rem(u, nc)
                stride = nrows // NS
                base = row0 + SH + j * BLK
                back = jnp.where(j == nc - 1, nrows, 0)
                src = [[h.at[b, g] for b in range(B)] for h in (k_hbm, v_hbm)]
                dst = [[h.at[slot, b] for b in range(B)] for h in (k_buf, v_buf)]

                def block(w, b, s, prio):
                    out = []
                    for o, r in pieces(s == NS - 1):
                        row = base + (s * stride + o)
                        if s == NS - 1 and SH and o >= BLK - SH:
                            row = row - back
                        out.append((pltpu.make_async_copy(
                            src[w][b].at[pl.ds(pl.multiple_of(row, 16), r)],
                            dst[w][b].at[pl.ds(s * BLK + o, r)],
                            kv_sem.at[slot, w]), prio))
                    return out

                def go(l0, l1):
                    for i in range(max(len(l0), len(l1))):
                        for l in (l0, l1):
                            if i < len(l):
                                l[i][0].start(priority=l[i][1])

                ss = list(range(NS))
                if rev:
                    ss = ss[0::2] + ss[1::2]
                if mode == "kv":
                    for s in ss:
                        for b in range(B):
                            go(block(0, b, s, 0), block(1, b, s, 1))
                elif mode == "bb":
                    for s in ss:
                        for w in range(2):
                            go(block(w, 0, s, 0), block(w, 1, s, 1))

            wcuts = sorted({0, HD // 2} | ({HD - WSH} if WSH else set())) + [HD]

            def wblock(src, dst, sem, blk, prio):
                out = []
                nxt = jnp.where(blk == nwb - 1, 0, blk + 1)
                for lo, hi in zip(wcuts[:-1], wcuts[1:]):
                    rg, c = (blk, WSH + lo) if WSH + lo < HD else (nxt, WSH + lo - HD)
                    r0 = pl.multiple_of(rg * WB, WB)
                    out.append((pltpu.make_async_copy(
                        src.at[pl.ds(r0, WB), pl.ds(c, hi - lo)],
                        dst.at[pl.ds(r0, WB), pl.ds(c, hi - lo)], sem(rg)), prio))
                return out

            def start_rows(src, dst, sem, first, count, nstream):
                per = count // nstream

                def wrap(blk):
                    return jnp.where(blk < 0, blk + nwb, blk)

                def body(i, _):
                    half = nstream // 2
                    for s in range(half):
                        l0 = wblock(src, dst, sem, wrap(first + s * per + i), 0)
                        l1 = wblock(src, dst, sem, wrap(first + (s + half) * per + i), 1)
                        for x, y in zip(l0, l1):
                            x[0].start(priority=x[1])
                            y[0].start(priority=y[1])
                lax.fori_loop(0, per, body, None)

            tiles = [(lo, min(lo + 128, D)) for lo in range(0, D, 128)]

            def start_woa(n):
                lo, hi = tiles[n]
                start_rows(woa_hbm, wo_buf.at[0], lambda rg: woa_sem.at[lax.div(rg, 128 // WB)],
                           lo // WB - (1 if WSH else 0), (hi - lo) // WB, 4)

            def start_step(t):
                slot = lax.rem(t, R)

                @pl.when(t < NB_)
                def _():
                    start_chunk(1, t, slot)

                @pl.when(jnp.logical_and(t >= NB_, t < NTOT))
                def _():
                    start_chunk(0, t - NB_, slot)

                for n in range(min(R - 1, len(tiles))):
                    pl.when(t == NTOT + n)(lambda n=n: start_woa(n))

            x_copies = [
                pltpu.make_async_copy(xa_hbm, x_buf.at[0], x_sem.at[0]),
                pltpu.make_async_copy(xb_hbm, x_buf.at[1], x_sem.at[1]),
            ]
            start_rows(wqb_hbm, wq_buf.at[1], lambda rg: w_sem.at[1], 0, nwb, 8)
            for c in x_copies:
                c.start()
            start_rows(wqa_hbm, wq_buf.at[0], lambda rg: w_sem.at[0], 0, nwb, 8)
            start_rows(wob_hbm, wo_buf.at[1], lambda rg: w_sem.at[2], 0, nwb, 8)

            def warm(t, _):
                start_chunk(1, t, t)
            lax.fori_loop(0, R - 1, warm, None)

            def row_ids(n):
                return lax.broadcasted_iota(jnp.int32, (_ROWS, n), 0)

            def project_q(br):
                x_copies[br].wait()
                x = x_buf[br].astype(jnp.float32)
                xr = jnp.where(row_ids(D) % 2 == 0,
                               jnp.broadcast_to(x[0:1], (_ROWS, D)),
                               jnp.broadcast_to(x[1:2], (_ROWS, D))).astype(jnp.bfloat16)
                pltpu.make_async_copy(wq_buf.at[br], wq_buf.at[br], w_sem.at[br]).wait()

                def body(g, _):
                    cols = pl.ds(pl.multiple_of(g * GW, GW), GW)
                    q = lax.dot_general(xr, wq_buf[br, :, cols], _NN,
                                        preferred_element_type=jnp.float32)
                    q_scr[br, g] = jnp.where((row_ids(Dh) // 2) % 2 == 0, q[:, :Dh], q[:, Dh:])
                lax.fori_loop(0, Hkv, body, None)

            def attend(br, first):
                nc = branches[br][2]

                def group_body(g, _):
                    q = q_scr[br, g].astype(jnp.bfloat16)

                    def chunk_body(j, carry):
                        m, l, acc = carry
                        t = first + g * nc + j
                        slot = lax.rem(t, R)
                        start_step(t + (R - 1))
                        pltpu.make_async_copy(k_buf.at[slot], k_buf.at[slot], kv_sem.at[slot, 0]).wait()
                        pltpu.make_async_copy(v_buf.at[slot], v_buf.at[slot], kv_sem.at[slot, 1]).wait()
                        s0, s1 = [lax.dot_general(q, k_buf[slot, b], _NT,
                                                  preferred_element_type=jnp.float32) for b in range(B)]
                        s = jnp.where(row_ids(CH) % 2 == 0, s0, s1) * scale
                        m_new = jnp.maximum(m, jnp.max(s, axis=-1, keepdims=True))
                        alpha = jnp.exp(m - m_new)
                        p = jnp.exp(s - m_new)
                        l = alpha * l + jnp.sum(p, axis=-1, keepdims=True)
                        pb = p.astype(jnp.bfloat16)
                        o0, o1 = [lax.dot_general(pb, v_buf[slot, b], _NN,
                                                  preferred_element_type=jnp.float32) for b in range(B)]
                        acc = alpha * acc + jnp.where(row_ids(Dh) % 2 == 0, o0, o1)
                        return m_new, l, acc

                    init = (jnp.full((_ROWS, 1), -jnp.inf, jnp.float32),
                            jnp.zeros((_ROWS, 1), jnp.float32),
                            jnp.zeros((_ROWS, Dh), jnp.float32))
                    _, l, acc = lax.fori_loop(0, nc, chunk_body, init)
                    o = acc / l
                    c0 = pl.multiple_of(g * GW, GW)
                    o_scr[br, :, pl.ds(c0, Dh)] = o
                    o_scr[br, :, pl.ds(c0 + Dh, Dh)] = pltpu.roll(o, _ROWS - 2, 0)

                lax.fori_loop(0, Hkv, group_body, None)

            project_q(1)
            project_q(0)
            attend(1, 0)
            pltpu.make_async_copy(wo_buf.at[1], wo_buf.at[1], w_sem.at[2]).wait()
            res = lax.dot_general(o_scr[1].astype(jnp.bfloat16), wo_buf[1], _NT,
                                  preferred_element_type=jnp.float32)
            out_ref[:, D:2 * D] = res[0:B].astype(out_ref.dtype)
            attend(0, NB_)
            for n in range(R - 1, len(tiles)):
                start_woa(n)
            oa = o_scr[0].astype(jnp.bfloat16)
            for n, (lo, hi) in enumerate(tiles):
                piece = wo_buf.at[0, pl.ds(lo, hi - lo)]
                pltpu.make_async_copy(piece, piece, woa_sem.at[n]).wait()
                res = lax.dot_general(oa, piece[...], _NT, preferred_element_type=jnp.float32)
                out_ref[:, lo:hi] = res[0:B].astype(out_ref.dtype)

        hbm = pl.BlockSpec(memory_space=pltpu.HBM)
        out = pl.pallas_call(
            kernel,
            out_shape=jax.ShapeDtypeStruct((B, 2 * D), A_x.dtype),
            in_specs=[hbm] * 10,
            out_specs=pl.BlockSpec(memory_space=pltpu.VMEM),
            scratch_shapes=[
                pltpu.VMEM((R, B, CH, Dh), A_k_cache.dtype),
                pltpu.VMEM((R, B, CH, Dh), A_v_cache.dtype),
                pltpu.VMEM((2, B, D), A_x.dtype),
                pltpu.VMEM((2, D, HD), A_wq.dtype),
                pltpu.VMEM((2, D, HD), A_wo.dtype),
                pltpu.VMEM((2, Hkv, _ROWS, Dh), jnp.float32),
                pltpu.VMEM((2, _ROWS, HD), jnp.float32),
                pltpu.SemaphoreType.DMA((R, 2)),
                pltpu.SemaphoreType.DMA((2,)),
                pltpu.SemaphoreType.DMA((3,)),
                pltpu.SemaphoreType.DMA((4,)),
            ],
            compiler_params=pltpu.CompilerParams(vmem_limit_bytes=100 * 2**20, disable_bounds_checks=nobc),
            name=name,
        )(A_x.reshape(B, D), A_k_cache, A_v_cache, A_wq, A_wo.T,
          B_x.reshape(B, D), B_k_cache, B_v_cache, B_wq, B_wo.T)
        return out.reshape(B, Sq, 2 * D)
    return jax.jit(fn)


pallas_concat_heads__gqa_block_cached__sliding_block_cached__decode_kernel = build(R=5,SH=64,WSH=2048)
```

```python
import jax
import jax.numpy as jnp
import numpy as np
from jax import lax
import jax.experimental.pallas as pl
import jax.experimental.pallas.tpu as pltpu

_NN = (((1,), (0,)), ((), ()))
_NT = (((1,), (1,)), ((), ()))

_HQ, _DH = 16, 256
_ROWS = 8
_F32_MIN = float(np.finfo(np.float32).min)

_SEGS = 4
_BLOCK = 128
_COPY = 64
_PHASE = 64
_SLOTS = 5
_WROWS = 8
_WSTRIDE = 9
_LANES = 128


def _row_ids(n):
    return lax.broadcasted_iota(jnp.int32, (_ROWS, n), 0)


def _dot(a, b, dims):
    return lax.dot_general(a, b, dims, preferred_element_type=jnp.float32)


def _kernel(xa_hbm, ka_hbm, va_hbm, wqa_hbm, woa_hbm,
            xb_hbm, kb_hbm, vb_hbm, wqb_hbm, wob_hbm, out_ref,
            kv_buf, x_buf, wq_buf, wo_buf, q_scr, o_scr,
            kv_sem, head_sem, tail_sem):
    batch, hkv, _, _, dh = ka_hbm.shape
    d_model, hd = wqa_hbm.shape
    gw = hd // hkv
    scale = dh ** -0.5
    keys = _SEGS * _BLOCK
    n_wblk = d_model // _WROWS

    A, B = 0, 1
    caches = ((ka_hbm, va_hbm), (kb_hbm, vb_hbm))
    seg_rows = [k.shape[3] for k, _ in caches]
    seg_first = [k.shape[2] - _SEGS for k, _ in caches]
    chunks = [rows // _BLOCK for rows in seg_rows]
    steps_b = hkv * chunks[B]
    steps = steps_b + hkv * chunks[A]

    def start_kv(br, u, slot):
        g, j = lax.div(u, chunks[br]), lax.rem(u, chunks[br])
        first = _PHASE + j * _BLOCK
        wrap = jnp.where(j == chunks[br] - 1, seg_rows[br], 0)
        for s in (*range(0, _SEGS, 2), *range(1, _SEGS, 2)):
            for b in range(batch):
                for o in range(0, _BLOCK, _COPY):
                    row = first + o - (wrap if o >= _BLOCK - _PHASE else 0)
                    rows = pl.ds(pl.multiple_of(row, _COPY), _COPY)
                    for kv in range(2):
                        pltpu.make_async_copy(
                            caches[br][kv].at[b, g, seg_first[br] + s, rows],
                            kv_buf.at[slot, kv, b, pl.ds(s * _BLOCK + o, _COPY)],
                            kv_sem.at[slot]).start(priority=kv)

    def start_weight_blocks(blocks):
        cols = hd * _COPY // _BLOCK
        first = hd * _PHASE // _BLOCK
        for c in range(first, first + hd, cols):
            for src, dst, sem_of, blk, thread in blocks:
                grp = blk + c // hd
                grp = jnp.where(grp < 0, grp + n_wblk, grp)
                grp = jnp.where(grp >= n_wblk, grp - n_wblk, grp)
                idx = (pl.ds(pl.multiple_of(grp * _WROWS, _WROWS), _WROWS),
                       pl.ds(c % hd, cols))
                pltpu.make_async_copy(
                    src.at[idx], dst.at[idx], sem_of(grp)).start(priority=thread)

    tiles = [(lo, min(lo + _LANES, d_model)) for lo in range(0, d_model, _LANES)]

    def tail_sem_of(grp):
        return tail_sem.at[lax.div(grp, _LANES // _WROWS)]

    def start_tail(n):
        lo, hi = (edge // _WROWS for edge in tiles[n])
        quarter = (hi - lo) // 4
        lo -= 1 if _PHASE else 0
        thread = 1 if n == len(tiles) - 1 else 0

        @pl.loop(0, quarter)
        def _(i):
            for k in range(2):
                start_weight_blocks([
                    (woa_hbm, wo_buf.at[A], tail_sem_of, lo + k * quarter + i, thread),
                    (woa_hbm, wo_buf.at[A], tail_sem_of, lo + (k + 2) * quarter + i, 1)])

    def start_step(t, br):
        slot = lax.rem(t, _SLOTS)
        if br == B:
            pl.when(t < steps_b)(lambda: start_kv(B, t, slot))
        pl.when(jnp.logical_and(t >= steps_b, t < steps))(
            lambda: start_kv(A, t - steps_b, slot))
        if br == A:
            for n in range(len(tiles)):
                pl.when(t == steps + n)(lambda n=n: start_tail(n))

    def wait_filled(ref, sem):
        pltpu.make_async_copy(ref, ref, sem).wait()

    head = ((wqb_hbm, wq_buf.at[B]), (wqa_hbm, wq_buf.at[A]), (wob_hbm, wo_buf.at[B]))

    @pl.loop(0, n_wblk // 2)
    def _(i):
        blocks = [(src, dst, lambda _: head_sem, lax.rem((2 * i + k) * _WSTRIDE, n_wblk))
                  for k in range(2) for src, dst in head]
        for p in range(0, len(blocks), 2):
            start_weight_blocks([blocks[p] + (0,), blocks[p + 1] + (1,)])

    x_copies = [pltpu.make_async_copy(src, x_buf.at[br], head_sem)
                for br, src in ((A, xa_hbm), (B, xb_hbm))]
    for copy in x_copies:
        copy.start()

    @pl.loop(0, _SLOTS - 1)
    def _(t):
        start_kv(B, t, t)

    for copy in x_copies:
        copy.wait()
    for _, dst in head:
        wait_filled(dst, head_sem)

    @pl.loop(0, 2)
    def _(br):
        x = x_buf[br].astype(jnp.float32)
        x = jnp.where(_row_ids(d_model) % 2 == 0,
                      jnp.broadcast_to(x[0:1], (_ROWS, d_model)),
                      jnp.broadcast_to(x[1:2], (_ROWS, d_model))).astype(x_buf.dtype)

        @pl.loop(0, hkv)
        def _(g):
            q = _dot(x, wq_buf[br, :, pl.ds(pl.multiple_of(g * gw, gw), gw)], _NN)
            q_scr[br, g] = jnp.where((_row_ids(dh) // 2) % 2 == 0, q[:, :dh], q[:, dh:])

    def attend(br, first_step):
        @pl.loop(0, hkv)
        def _(g):
            q = q_scr[br, g].astype(kv_buf.dtype)

            def step(j, carry):
                m, l, acc = carry
                t = first_step + g * chunks[br] + j
                slot = lax.rem(t, _SLOTS)
                start_step(t + _SLOTS - 1, br)
                wait_filled(kv_buf.at[slot], kv_sem.at[slot])
                s0, s1 = (_dot(q, kv_buf[slot, 0, b], _NT) for b in range(batch))
                s = jnp.where(_row_ids(keys) % 2 == 0, s0, s1) * scale
                m_new = jnp.maximum(m, jnp.max(s, axis=-1, keepdims=True))
                alpha = jnp.exp(m - m_new)
                p = jnp.exp(s - m_new)
                l = alpha * l + jnp.sum(p, axis=-1, keepdims=True)
                p = p.astype(kv_buf.dtype)
                o0, o1 = (_dot(p, kv_buf[slot, 1, b], _NN) for b in range(batch))
                return m_new, l, alpha * acc + jnp.where(_row_ids(dh) % 2 == 0, o0, o1)

            _, l, acc = lax.fori_loop(0, chunks[br], step, (
                jnp.full((_ROWS, 1), _F32_MIN, jnp.float32),
                jnp.zeros((_ROWS, 1), jnp.float32),
                jnp.zeros((_ROWS, dh), jnp.float32)))
            o = acc / l
            col = pl.multiple_of(g * gw, gw)
            o_scr[:, pl.ds(col, dh)] = o
            o_scr[:, pl.ds(col + dh, dh)] = pltpu.roll(o, _ROWS - batch, 0)

        return o_scr[...].astype(wo_buf.dtype)

    o_b = attend(B, 0)
    out_ref[:, d_model:] = _dot(o_b, wo_buf[B], _NT)[:batch].astype(out_ref.dtype)

    o_a = attend(A, steps_b)
    for n, (lo, hi) in enumerate(tiles):
        piece = wo_buf.at[A, pl.ds(lo, hi - lo)]
        wait_filled(piece, tail_sem.at[n])
        out_ref[:, lo:hi] = _dot(o_a, piece[...], _NT)[:batch].astype(out_ref.dtype)


@jax.jit
def pallas_concat_heads__gqa_block_cached__sliding_block_cached__decode_kernel(
    A_x: jax.Array,
    A_k_cache: jax.Array,
    A_v_cache: jax.Array,
    A_wq: jax.Array,
    A_wo: jax.Array,
    B_x: jax.Array,
    B_k_cache: jax.Array,
    B_v_cache: jax.Array,
    B_wq: jax.Array,
    B_wo: jax.Array,
):
    batch, sq, d_model = A_x.shape
    _, hkv, sk_a, dh = A_k_cache.shape
    sk_b = B_k_cache.shape[2]
    window = min(4096, max(256, sk_b // 4))
    hd = _HQ * _DH
    keys = _SEGS * _BLOCK
    n_tiles = pl.cdiv(d_model, _LANES)
    assert (batch, sq, dh, _HQ // hkv) == (2, 1, _DH, 2)
    assert sk_a % keys == 0 and window % keys == 0 and sk_b % window == 0
    assert hkv * (window // keys) >= _SLOTS > n_tiles
    assert d_model % (4 * _WROWS) == 0 and np.gcd(_WSTRIDE, d_model // _WROWS) == 1
    dtype = A_x.dtype

    def segments(cache, rows):
        return cache.reshape(batch, hkv, -1, rows // _SEGS, dh)

    out = pl.pallas_call(
        _kernel,
        out_shape=jax.ShapeDtypeStruct((batch, 2 * d_model), dtype),
        in_specs=[pl.BlockSpec(memory_space=pltpu.HBM)] * 10,
        out_specs=pl.BlockSpec(memory_space=pltpu.VMEM),
        scratch_shapes=[
            pltpu.VMEM((_SLOTS, 2, batch, keys, dh), dtype),
            pltpu.VMEM((2, batch, d_model), dtype),
            pltpu.VMEM((2, d_model, hd), dtype),
            pltpu.VMEM((2, d_model, hd), dtype),
            pltpu.VMEM((2, hkv, _ROWS, dh), jnp.float32),
            pltpu.VMEM((_ROWS, hd), jnp.float32),
            pltpu.SemaphoreType.DMA((_SLOTS,)),
            pltpu.SemaphoreType.DMA(()),
            pltpu.SemaphoreType.DMA((n_tiles,)),
        ],
        compiler_params=pltpu.CompilerParams(vmem_limit_bytes=48 * 2**20),
        name="concat_gqa_sliding_decode",
    )(A_x.reshape(batch, d_model), segments(A_k_cache, sk_a), segments(A_v_cache, sk_a),
      A_wq, A_wo.T,
      B_x.reshape(batch, d_model), segments(B_k_cache, window), segments(B_v_cache, window),
      B_wq, B_wo.T)
    return out.reshape(batch, sq, 2 * d_model)
```
